```python
import os as _os
_os.environ.setdefault("JAX_PLATFORMS", "cpu")
import jax
import jax.numpy as jnp

def _softmax(x, axis=-1):
    return jax.nn.softmax(x, axis=axis)
def _gelu(x):
    return jax.nn.gelu(x, approximate=True)
def _silu(x):
    return jax.nn.silu(x)
def _sigmoid(x):
    return jax.nn.sigmoid(x)
def _layernorm(x, axis=-1, eps=1e-5):
    m = jnp.mean(x, axis=axis, keepdims=True)
    v = jnp.var(x, axis=axis, keepdims=True)
    return (x - m) / jnp.sqrt(v + eps)
def _scatter_add(tgt, idx, src, axis=0):
    return tgt.at[idx].add(src)
def _segment_sum(src, seg, n):
    return jax.ops.segment_sum(src, seg, n)
class _Rng:
    def __init__(self, key):
        self._k = key
    def _next(self):
        self._k, sub = jax.random.split(self._k)
        return sub
    def normal(self, shape):
        return jax.random.normal(self._next(), shape, dtype=jnp.bfloat16)
    def randint(self, lo, hi, shape):
        return jax.random.randint(self._next(), shape, lo, hi, dtype=jnp.int32)
    def uniform(self, shape, lo=0.0, hi=1.0):
        return jax.random.uniform(self._next(), shape, jnp.bfloat16, lo, hi)
    def permutation(self, n):
        return jax.random.permutation(self._next(), n)


kernel_name = 'concat_heads__mha_block_cached__mha_block_cached__near_ridge'

def setup_inputs():
    _rng = _Rng(jax.random.key(int.from_bytes(__import__("os").urandom(4), "little")))
    _w = (lambda a: (lambda t: t.astype(jnp.bfloat16) if jnp.issubdtype(t.dtype, jnp.floating) else t)(jnp.asarray(a)))
    def _A_setup():
        B, Sq, D = 16, 192, 512
        H, Sk, Dh = 32, 512, 128
        return {
            "x": _w((lambda *s: _rng.normal(s) * 0.8)(B, Sq, D)),
            "k_cache": _w((lambda *s: _rng.normal(s) * 0.8)(B, H, Sk, Dh)),
            "v_cache": _w((lambda *s: _rng.normal(s) * 0.05)(B, H, Sk, Dh)),
            "wq": _w((lambda *s: _rng.normal(s) * 0.8)(D, H * Dh) * (D ** -0.5)),
            "wo": _w((lambda *s: _rng.normal(s) * 0.05)(H * Dh, D) * ((H * Dh) ** -0.5)),
        }
    _A_in = _A_setup()

    def _B_setup():
        B, Sq, D = 16, 192, 512
        H, Sk, Dh = 32, 512, 128
        return {
            "x": _w((lambda *s: _rng.normal(s) * 0.8)(B, Sq, D)),
            "k_cache": _w((lambda *s: _rng.normal(s) * 0.8)(B, H, Sk, Dh)),
            "v_cache": _w((lambda *s: _rng.normal(s) * 0.05)(B, H, Sk, Dh)),
            "wq": _w((lambda *s: _rng.normal(s) * 0.8)(D, H * Dh) * (D ** -0.5)),
            "wo": _w((lambda *s: _rng.normal(s) * 0.05)(H * Dh, D) * ((H * Dh) ** -0.5)),
        }
    _B_in = _B_setup()

    return {
        "A_x": _A_in["x"],
        "A_k_cache": _A_in["k_cache"],
        "A_v_cache": _A_in["v_cache"],
        "A_wq": _A_in["wq"],
        "A_wo": _A_in["wo"],
        "B_x": _B_in["x"],
        "B_k_cache": _B_in["k_cache"],
        "B_v_cache": _B_in["v_cache"],
        "B_wq": _B_in["wq"],
        "B_wo": _B_in["wo"],
    }

def reference(A_x, A_k_cache, A_v_cache, A_wq, A_wo, B_x, B_k_cache, B_v_cache, B_wq, B_wo):
    def _A_ref(x, k_cache, v_cache, wq, wo):
        B, Sq, D = x.shape
        H, Dh = 32, 128
        q = (lambda x, *d: x.transpose(*d))((x @ wq).reshape(B, Sq, H, Dh), 0, 2, 1, 3)
        scores = jnp.einsum("bhqd,bhkd->bhqk", q, k_cache) * (Dh ** -0.5)
        p = _softmax(scores, axis=-1)
        o = jnp.einsum("bhqk,bhkd->bhqd", p, v_cache)
        return (lambda x, *d: x.transpose(*d))(o, 0, 2, 1, 3).reshape(B, Sq, H * Dh) @ wo

    def _B_ref(x, k_cache, v_cache, wq, wo):
        B, Sq, D = x.shape
        H, Dh = 32, 128
        q = (lambda x, *d: x.transpose(*d))((x @ wq).reshape(B, Sq, H, Dh), 0, 2, 1, 3)
        scores = jnp.einsum("bhqd,bhkd->bhqk", q, k_cache) * (Dh ** -0.5)
        p = _softmax(scores, axis=-1)
        o = jnp.einsum("bhqk,bhkd->bhqd", p, v_cache)
        return (lambda x, *d: x.transpose(*d))(o, 0, 2, 1, 3).reshape(B, Sq, H * Dh) @ wo

    a = _A_ref(A_x, A_k_cache, A_v_cache, A_wq, A_wo)
    b = _B_ref(B_x, B_k_cache, B_v_cache, B_wq, B_wo)
    return jnp.concatenate([a, b], axis=-1)
```

```python
import functools
import jax
import jax.numpy as jnp
from jax import lax
import jax.experimental.pallas as pl
import jax.experimental.pallas.tpu as pltpu

B, SQ, D = 16, 192, 512
H, SK, DH = 32, 512, 128
NU = 2 * B
L = 5
NQ = 8
NKV = 4
WC = 8
HC = H // WC
LOG2E = 1.4426950408889634
QSCALE = (DH ** -0.5) * LOG2E
F32 = jnp.float32
BF16 = jnp.bfloat16


def qproj(x, wq_h):
    q = jnp.dot(x, wq_h, preferred_element_type=F32)
    return (q * QSCALE).astype(BF16)


def qk(q, k):
    return lax.dot_general(q, k, (((1,), (1,)), ((), ())), preferred_element_type=F32)


def softmax_pv(s, v):
    m = jnp.max(s, axis=-1, keepdims=True)
    p = jnp.exp2(s - m)
    l = jnp.sum(p, axis=-1, keepdims=True)
    o = jnp.dot(p.astype(BF16), v, preferred_element_type=F32)
    r = pl.reciprocal(l, approx=True)
    r = r * (2.0 - l * r)
    return (o * r).astype(BF16)


def kernel(xa, ka, va, wqa, woa, xb, kb, vb, wqb, wob, out,
           kbuf, vbuf, xbuf, wq, wo, qbuf, acc, ol, obuf, kv_sem, w_sem, wq_sem, o_sem, ord_sem):
    i = pl.program_id(0)

    def kv_copies(src_k, src_v, b, s):
        return (pltpu.make_async_copy(src_k.at[b], kbuf.at[s], kv_sem.at[0, s]),
                pltpu.make_async_copy(src_v.at[b], vbuf.at[s], kv_sem.at[1, s]))

    def start_kv(u):
        s = u & (NKV - 1)
        b = u & (B - 1)

        @pl.when(u < B)
        def _():
            for c in kv_copies(ka, va, b, s):
                c.start()

        @pl.when(u >= B)
        def _():
            for c in kv_copies(kb, vb, b, s):
                c.start()

    def wait_kv(s):
        for c in kv_copies(ka, va, 0, s):
            c.wait()

    def wq_chunk(c):
        cols = pl.ds(pl.multiple_of(c * (HC * DH), HC * DH), HC * DH)
        return pltpu.make_async_copy(wqa.at[:, cols], wq.at[0, :, cols], wq_sem.at[c])

    x0_copy = pltpu.make_async_copy(xa.at[pl.ds(0, L + 1)], xbuf.at[pl.ds(0, L + 1)], w_sem.at[0])
    woa_copy = pltpu.make_async_copy(woa, wo.at[0], w_sem.at[1])
    x1_copy = pltpu.make_async_copy(xa.at[pl.ds(L + 1, B - L - 1)], xbuf.at[pl.ds(L + 1, B - L - 1)], w_sem.at[2])
    wqb_copy = pltpu.make_async_copy(wqb, wq.at[1], w_sem.at[3])
    wob_copy = pltpu.make_async_copy(wob, wo.at[1], w_sem.at[4])
    xb_copy = pltpu.make_async_copy(xb, xbuf.at[pl.ds(B, B)], w_sem.at[5])

    def out_copy(u):
        s = u & 1
        col = pl.multiple_of((u >> 4) * D, D)
        return pltpu.make_async_copy(obuf.at[s], out.at[u & (B - 1), :, pl.ds(col, D)], o_sem.at[s])

    @pl.when(i == 0)
    def _():
        def fence():
            pl.semaphore_signal(ord_sem, 1)
            pl.semaphore_wait(ord_sem, 1)

        order = [x0_copy] + [wq_chunk(c) for c in range(WC)]
        order += list(kv_copies(ka, va, 0, 0)) + [woa_copy, x1_copy]
        for u in range(1, NKV):
            order += list(kv_copies(ka, va, u, u))
        order += [wqb_copy, wob_copy, xb_copy]
        for c in order:
            c.start()
            fence()
        acc[...] = jnp.zeros_like(acc)
        ol[...] = jnp.zeros_like(ol)
        x0_copy.wait()

        def qphase(c, carry):
            wq_chunk(c).wait()
            for u in range(L):
                x = xbuf[u]
                for hh in range(HC):
                    h = c * HC + hh
                    col = pl.multiple_of(h * DH, DH)
                    qbuf[u, h] = qproj(x, wq[0, :, pl.ds(col, DH)])
            return carry

        lax.fori_loop(0, WC, qphase, 0)
        woa_copy.wait()

    @pl.when(i == 1)
    def _():
        x1_copy.wait()

    @pl.when(i == B - L)
    def _():
        wqb_copy.wait()
        xb_copy.wait()

    @pl.when(i == B)
    def _():
        wob_copy.wait()

    kslot = i & (NKV - 1)
    wait_kv(kslot)

    br = i >> 4
    br_p = jnp.maximum(i - 1, 0) >> 4
    qslot = i & (NQ - 1)

    def o_proj(h, o_prev):
        if h == 0:
            fin = acc[...] + jnp.dot(ol[...], wo[br_p, (H - 1) * DH:H * DH, :], preferred_element_type=F32)
            obuf[(i + 1) & 1] = fin.astype(BF16)
        elif h == 1:
            acc[...] = jnp.dot(o_prev, wo[br, 0:DH, :], preferred_element_type=F32)
        else:
            acc[...] += jnp.dot(o_prev, wo[br, (h - 1) * DH:h * DH, :], preferred_element_type=F32)

    def body(with_q):
        if with_q:
            un = i + L
            br_n = un >> 4
            qslot_n = un & (NQ - 1)
            x = xbuf[un]
        o_prev = None
        for h in range(H):
            if with_q and h == 0:
                o_proj(0, None)
            s = qk(qbuf[qslot, h], kbuf[kslot, h])
            if with_q and h == 0:
                qbuf[qslot_n, h] = qproj(x, wq[br_n, :, h * DH:(h + 1) * DH])
            else:
                o_proj(h, o_prev)
            o_prev = softmax_pv(s, vbuf[kslot, h])
            if with_q and h > 0:
                qbuf[qslot_n, h] = qproj(x, wq[br_n, :, h * DH:(h + 1) * DH])
        ol[...] = o_prev

    @pl.when(i < NU - L)
    def _():
        body(True)

    @pl.when(i >= NU - L)
    def _():
        body(False)

    @pl.when(i + NKV < NU)
    def _():
        start_kv(i + NKV)

    @pl.when(i >= 1)
    def _():
        out_copy(i - 1).start()

    @pl.when(i >= 2)
    def _():
        out_copy(i - 2).wait()

    @pl.when(i == NU - 1)
    def _():
        fin = acc[...] + jnp.dot(ol[...], wo[1, (H - 1) * DH:H * DH, :], preferred_element_type=F32)
        obuf[(NU - 1) % 2] = fin.astype(BF16)
        out_copy(NU - 1).start()
        out_copy(NU - 2).wait()
        out_copy(NU - 1).wait()


@jax.jit
def pallas_concat_heads__mha_block_cached__mha_block_cached__near_ridge_kernel(
    A_x, A_k_cache, A_v_cache, A_wq, A_wo, B_x, B_k_cache, B_v_cache, B_wq, B_wo):
    any_spec = pl.BlockSpec(memory_space=pl.ANY)
    return pl.pallas_call(
        kernel,
        grid=(NU,),
        in_specs=[any_spec] * 10,
        out_specs=any_spec,
        out_shape=jax.ShapeDtypeStruct((B, SQ, 2 * D), jnp.bfloat16),
        scratch_shapes=[
            pltpu.VMEM((NKV, H, SK, DH), BF16),
            pltpu.VMEM((NKV, H, SK, DH), BF16),
            pltpu.VMEM((NU, SQ, D), BF16),
            pltpu.VMEM((2, D, H * DH), BF16),
            pltpu.VMEM((2, H * DH, D), BF16),
            pltpu.VMEM((NQ, H, SQ, DH), BF16),
            pltpu.VMEM((SQ, D), F32),
            pltpu.VMEM((SQ, DH), BF16),
            pltpu.VMEM((2, SQ, D), BF16),
            pltpu.SemaphoreType.DMA((2, NKV)),
            pltpu.SemaphoreType.DMA((6,)),
            pltpu.SemaphoreType.DMA((WC,)),
            pltpu.SemaphoreType.DMA((2,)),
            pltpu.SemaphoreType.REGULAR,
        ],
        compiler_params=pltpu.CompilerParams(
            dimension_semantics=("arbitrary",),
            vmem_limit_bytes=110 * 1024 * 1024,
            disable_bounds_checks=True),
    )(A_x, A_k_cache, A_v_cache, A_wq, A_wo, B_x, B_k_cache, B_v_cache, B_wq, B_wo)
```

```python
import jax
import jax.numpy as jnp
from jax import lax
import jax.experimental.pallas as pl
import jax.experimental.pallas.tpu as pltpu

B, SQ, D = 16, 192, 512
H, SK, DH = 32, 512, 128
NU = 2 * B
L = 7
NQ = 8
NKV = 4
HC0 = 4
WC = 4
HC = (H - HC0) // WC
LOG2E = 1.4426950408889634
QSCALE = (DH ** -0.5) * LOG2E
F32 = jnp.float32
BF16 = jnp.bfloat16


def _qproj(x, wq_h):
    q = jnp.dot(x, wq_h, preferred_element_type=F32)
    return (q * QSCALE).astype(BF16)


def _qk(q, k):
    return lax.dot_general(q, k, (((1,), (1,)), ((), ())), preferred_element_type=F32)


def _softmax_pv(s, v):
    m = jnp.max(s, axis=-1, keepdims=True)
    p = jnp.exp2(s - m)
    l = jnp.sum(p, axis=-1, keepdims=True)
    o = jnp.dot(p.astype(BF16), v, preferred_element_type=F32)
    r = pl.reciprocal(l, approx=True)
    r = r * (2.0 - l * r)
    return (o * r).astype(BF16)


def _kernel(xa, ka, va, wqa, woa, xb, kb, vb, wqb, wob, out,
            kvbuf, xbuf, wq, wo, qbuf, acc, ol, obuf, kv_sem, w_sem, wq_sem, o_sem, ord_sem):

    def kv_copies(src_k, src_v, b, s):
        return (pltpu.make_async_copy(src_k.at[b], kvbuf.at[s, 0], kv_sem.at[s]),
                pltpu.make_async_copy(src_v.at[b], kvbuf.at[s, 1], kv_sem.at[s]))

    def start_kv(u):
        s = u & (NKV - 1)
        b = u & (B - 1)

        @pl.when(u < B)
        def _():
            for c in kv_copies(ka, va, b, s):
                c.start()

        @pl.when(jnp.logical_and(u >= B, u < NU))
        def _():
            for c in kv_copies(kb, vb, b, s):
                c.start()

    def wait_kv(s):
        pltpu.make_async_copy(kvbuf.at[s], kvbuf.at[s], kv_sem.at[s]).wait()

    wq0_copy = pltpu.make_async_copy(wqa.at[:, pl.ds(0, HC0 * DH)], wq.at[0, :, pl.ds(0, HC0 * DH)], wq_sem.at[WC])

    def wq_chunk(c):
        cols = pl.ds(pl.multiple_of((HC0 + c * HC) * DH, DH), HC * DH)
        return pltpu.make_async_copy(wqa.at[:, cols], wq.at[0, :, cols], wq_sem.at[c])

    def xa_copy(lo, hi, sem):
        return pltpu.make_async_copy(xa.at[pl.ds(lo, hi - lo)], xbuf.at[pl.ds(lo, hi - lo)], sem)

    x0_copy = xa_copy(0, 1, w_sem.at[0])
    x1_copy = xa_copy(1, 3, w_sem.at[1])
    x2_copy = xa_copy(3, L, w_sem.at[2])
    x3_copy = xa_copy(L, B, w_sem.at[3])
    woa_copy = pltpu.make_async_copy(woa, wo.at[0], w_sem.at[4])
    wqb_copy = pltpu.make_async_copy(wqb, wq.at[1], w_sem.at[5])
    wob_copy = pltpu.make_async_copy(wob, wo.at[1], w_sem.at[6])
    xb_copy = pltpu.make_async_copy(xb, xbuf.at[pl.ds(B, B)], w_sem.at[7])

    def out_copy(u):
        col = pl.multiple_of((u >> 4) * D, D)
        return pltpu.make_async_copy(obuf.at[u], out.at[u & (B - 1), :, pl.ds(col, D)], o_sem)

    def fence():
        pl.semaphore_signal(ord_sem, 1)
        pl.semaphore_wait(ord_sem, 1)

    order = [x0_copy, wq0_copy, x1_copy, x2_copy] + [wq_chunk(c) for c in range(WC)]
    order += list(kv_copies(ka, va, 0, 0)) + [woa_copy, x3_copy]
    for u in range(1, NKV):
        order += list(kv_copies(ka, va, u, u))
    order += [wqb_copy, wob_copy, xb_copy]
    for c in order:
        c.start()
        fence()
    acc[...] = jnp.zeros_like(acc)
    ol[...] = jnp.zeros_like(ol)

    with jax.named_scope("x0wait"):
        x0_copy.wait()
        wq0_copy.wait()
    with jax.named_scope("q0"):
        for u in range(L):
            if u == 1:
                x1_copy.wait()
            if u == 3:
                x2_copy.wait()
            x = xbuf[u]
            for h in range(HC0):
                qbuf[u, h] = _qproj(x, wq[0, :, h * DH:(h + 1) * DH])

    def qphase(c, carry):
        wq_chunk(c).wait()
        for u in range(L):
            x = xbuf[u]
            for hh in range(HC):
                h = HC0 + c * HC + hh
                col = pl.multiple_of(h * DH, DH)
                qbuf[u, h] = _qproj(x, wq[0, :, pl.ds(col, DH)])
        return carry

    with jax.named_scope("qphase"):
        lax.fori_loop(0, WC, qphase, 0)
    with jax.named_scope("kv0wait"):
        woa_copy.wait()
        x3_copy.wait()
        wait_kv(0)

    def unit(i, br_p, with_q):
        kslot = i & (NKV - 1)
        br = i >> 4
        qslot = i & (NQ - 1)

        def o_last():
            fin = acc[...] + jnp.dot(ol[...], wo[br_p, (H - 1) * DH:H * DH, :], preferred_element_type=F32)
            obuf[jnp.maximum(i - 1, 0)] = fin.astype(BF16)

        def o_proj(h, o):
            r = jnp.dot(o, wo[br, h * DH:(h + 1) * DH, :], preferred_element_type=F32)
            if h == 0:
                acc[...] = r
            else:
                acc[...] += r

        def qk(h):
            return _qk(qbuf[qslot, h], kvbuf[kslot, 0, h])

        def pv(h, s):
            return _softmax_pv(s, kvbuf[kslot, 1, h])

        o = {}
        o_last()
        if with_q:
            un = i + L
            br_n = un >> 4
            qslot_n = un & (NQ - 1)
            x = xbuf[un]
            for h in range(H):
                s = qk(h)
                qbuf[qslot_n, h] = _qproj(x, wq[br_n, :, h * DH:(h + 1) * DH])
                o[h] = pv(h, s)
                if h >= 1:
                    o_proj(h - 1, o.pop(h - 1))
        else:
            s = {0: qk(0)}
            for h in range(H):
                if h + 1 < H:
                    s[h + 1] = qk(h + 1)
                o[h] = pv(h, s.pop(h))
                if h >= 1:
                    o_proj(h - 1, o.pop(h - 1))
        ol[...] = o.pop(H - 1)

        start_kv(i + NKV)

        @pl.when(i >= 1)
        def _():
            out_copy(i - 1).start()

        @pl.when(i + 1 < NU)
        def _():
            wait_kv((i + 1) & (NKV - 1))

        return br

    def full_body(i, br_p):
        with jax.named_scope("full"):
            return unit(i, br_p, True)

    def noq_body(i, br_p):
        with jax.named_scope("noq"):
            return unit(i, br_p, False)

    def segment(sg, br_p):
        lo = jnp.where(sg == 0, 0, B - L)
        hi = jnp.where(sg == 0, B - L, NU - L)
        br_p = lax.fori_loop(lo, hi, full_body, br_p)

        @pl.when(sg == 0)
        def _():
            wqb_copy.wait()
            xb_copy.wait()
            wob_copy.wait()

        return br_p

    br_p = lax.fori_loop(0, 2, segment, jnp.int32(0))
    lax.fori_loop(NU - L, NU, noq_body, br_p)

    fin = acc[...] + jnp.dot(ol[...], wo[1, (H - 1) * DH:H * DH, :], preferred_element_type=F32)
    obuf[NU - 1] = fin.astype(BF16)
    out_copy(NU - 1).start()
    pltpu.make_async_copy(obuf, obuf, o_sem).wait()


@jax.jit
def pallas_concat_heads__mha_block_cached__mha_block_cached__near_ridge_kernel(
    A_x, A_k_cache, A_v_cache, A_wq, A_wo, B_x, B_k_cache, B_v_cache, B_wq, B_wo):
    any_spec = pl.BlockSpec(memory_space=pl.ANY)
    return pl.pallas_call(
        _kernel,
        in_specs=[any_spec] * 10,
        out_specs=any_spec,
        out_shape=jax.ShapeDtypeStruct((B, SQ, 2 * D), jnp.bfloat16),
        scratch_shapes=[
            pltpu.VMEM((NKV, 2, H, SK, DH), BF16),
            pltpu.VMEM((NU, SQ, D), BF16),
            pltpu.VMEM((2, D, H * DH), BF16),
            pltpu.VMEM((2, H * DH, D), BF16),
            pltpu.VMEM((NQ, H, SQ, DH), BF16),
            pltpu.VMEM((SQ, D), F32),
            pltpu.VMEM((SQ, DH), BF16),
            pltpu.VMEM((NU, SQ, D), BF16),
            pltpu.SemaphoreType.DMA((NKV,)),
            pltpu.SemaphoreType.DMA((8,)),
            pltpu.SemaphoreType.DMA((WC + 1,)),
            pltpu.SemaphoreType.DMA,
            pltpu.SemaphoreType.REGULAR,
        ],
        compiler_params=pltpu.CompilerParams(
            vmem_limit_bytes=120 * 1024 * 1024,
            disable_bounds_checks=True),
    )(A_x, A_k_cache, A_v_cache, A_wq, A_wo, B_x, B_k_cache, B_v_cache, B_wq, B_wo)
```

```python
import jax
import jax.numpy as jnp
from jax import lax
import jax.experimental.pallas as pl
import jax.experimental.pallas.tpu as pltpu

B, SQ, D = 16, 192, 512
H, SK, DH = 32, 512, 128
NU = 2 * B
L = 7
NQ = 8
NKV = 4
HC0 = 4
WC = 2
HC = (H - HC0) // WC
LOG2E = 1.4426950408889634
QSCALE = (DH ** -0.5) * LOG2E
F32 = jnp.float32
BF16 = jnp.bfloat16


def _qproj(x, wq_h):
    q = jnp.dot(x, wq_h, preferred_element_type=F32)
    return (q * QSCALE).astype(BF16)


def _qk(q, k):
    return lax.dot_general(q, k, (((1,), (1,)), ((), ())), preferred_element_type=F32)


def _softmax_pv(s, v):
    m = jnp.max(s, axis=-1, keepdims=True)
    p = jnp.exp2(s - m)
    l = jnp.sum(p, axis=-1, keepdims=True)
    o = jnp.dot(p.astype(BF16), v, preferred_element_type=F32)
    r = pl.reciprocal(l, approx=True)
    r = r * (2.0 - l * r)
    return (o * r).astype(BF16)


def _kernel(xa, ka, va, wqa, woa, xb, kb, vb, wqb, wob, out,
            kvbuf, xbuf, wq, wo, qbuf, acc, ol, obuf, kv_sem, w_sem, wq_sem, o_sem, ord_sem):

    def kv_copies(src_k, src_v, b, s):
        return (pltpu.make_async_copy(src_k.at[b], kvbuf.at[s, 0], kv_sem.at[s]),
                pltpu.make_async_copy(src_v.at[b], kvbuf.at[s, 1], kv_sem.at[s]))

    def start_kv(u):
        s = u & (NKV - 1)
        b = u & (B - 1)

        @pl.when(u < B)
        def _():
            for c in kv_copies(ka, va, b, s):
                c.start()

        @pl.when(jnp.logical_and(u >= B, u < NU))
        def _():
            for c in kv_copies(kb, vb, b, s):
                c.start()

    def wait_kv(s):
        pltpu.make_async_copy(kvbuf.at[s], kvbuf.at[s], kv_sem.at[s]).wait()

    wq0_copy = pltpu.make_async_copy(wqa.at[:, pl.ds(0, HC0 * DH)], wq.at[0, :, pl.ds(0, HC0 * DH)], wq_sem.at[WC])

    def wq_chunk(c):
        cols = pl.ds(pl.multiple_of((HC0 + c * HC) * DH, DH), HC * DH)
        return pltpu.make_async_copy(wqa.at[:, cols], wq.at[0, :, cols], wq_sem.at[c])

    def xa_copy(lo, hi, sem):
        return pltpu.make_async_copy(xa.at[pl.ds(lo, hi - lo)], xbuf.at[pl.ds(lo, hi - lo)], sem)

    x0_copy = xa_copy(0, 1, w_sem.at[0])
    x1_copy = xa_copy(1, 3, w_sem.at[1])
    x2_copy = xa_copy(3, L, w_sem.at[2])
    x3_copy = xa_copy(L, B, w_sem.at[3])
    woa_copy = pltpu.make_async_copy(woa, wo.at[0], w_sem.at[4])
    wqb_copy = pltpu.make_async_copy(wqb, wq.at[1], w_sem.at[5])
    wob_copy = pltpu.make_async_copy(wob, wo.at[1], w_sem.at[6])
    xb_copy = pltpu.make_async_copy(xb, xbuf.at[pl.ds(B, B)], w_sem.at[7])

    def out_copy(u):
        col = pl.multiple_of((u >> 4) * D, D)
        return pltpu.make_async_copy(obuf.at[u], out.at[u & (B - 1), :, pl.ds(col, D)], o_sem)

    def fence():
        pl.semaphore_signal(ord_sem, 1)
        pl.semaphore_wait(ord_sem, 1)

    order = [x0_copy, wq0_copy, x1_copy, x2_copy] + [wq_chunk(c) for c in range(WC)]
    order += list(kv_copies(ka, va, 0, 0)) + [woa_copy, x3_copy]
    for u in range(1, NKV):
        order += list(kv_copies(ka, va, u, u))
    order += [wqb_copy, wob_copy, xb_copy]
    for c in order:
        c.start()
        fence()
    acc[...] = jnp.zeros_like(acc)
    ol[...] = jnp.zeros_like(ol)

    with jax.named_scope("x0wait"):
        x0_copy.wait()
        wq0_copy.wait()
    with jax.named_scope("q0"):
        for u in range(L):
            if u == 1:
                x1_copy.wait()
            if u == 3:
                x2_copy.wait()
            x = xbuf[u]
            for h in range(HC0):
                qbuf[u, h] = _qproj(x, wq[0, :, h * DH:(h + 1) * DH])

    def qphase(c, carry):
        wq_chunk(c).wait()
        for u in range(L):
            x = xbuf[u]
            for hh in range(HC):
                h = HC0 + c * HC + hh
                col = pl.multiple_of(h * DH, DH)
                qbuf[u, h] = _qproj(x, wq[0, :, pl.ds(col, DH)])
        return carry

    with jax.named_scope("qphase"):
        lax.fori_loop(0, WC, qphase, 0)
    with jax.named_scope("kv0wait"):
        woa_copy.wait()
        x3_copy.wait()
        wait_kv(0)

    def unit(i, br_p, with_q):
        kslot = i & (NKV - 1)
        br = i >> 4
        qslot = i & (NQ - 1)

        def o_last():
            fin = acc[...] + jnp.dot(ol[...], wo[br_p, (H - 1) * DH:H * DH, :], preferred_element_type=F32)
            obuf[jnp.maximum(i - 1, 0)] = fin.astype(BF16)

        def o_proj(h, o):
            r = jnp.dot(o, wo[br, h * DH:(h + 1) * DH, :], preferred_element_type=F32)
            if h == 0:
                acc[...] = r
            else:
                acc[...] += r

        def qk(h):
            return _qk(qbuf[qslot, h], kvbuf[kslot, 0, h])

        def pv(h, s):
            return _softmax_pv(s, kvbuf[kslot, 1, h])

        o = {}
        o_last()
        if with_q:
            un = i + L
            br_n = un >> 4
            qslot_n = un & (NQ - 1)
            x = xbuf[un]
            for h in range(H):
                s = qk(h)
                qbuf[qslot_n, h] = _qproj(x, wq[br_n, :, h * DH:(h + 1) * DH])
                o[h] = pv(h, s)
                if h >= 1:
                    o_proj(h - 1, o.pop(h - 1))
        else:
            s = {0: qk(0)}
            for h in range(H):
                if h + 1 < H:
                    s[h + 1] = qk(h + 1)
                o[h] = pv(h, s.pop(h))
                if h >= 1:
                    o_proj(h - 1, o.pop(h - 1))
        ol[...] = o.pop(H - 1)

        start_kv(i + NKV)

        @pl.when(i >= 1)
        def _():
            out_copy(i - 1).start()

        @pl.when(i + 1 < NU)
        def _():
            wait_kv((i + 1) & (NKV - 1))

        return br

    def full_body(i, br_p):
        with jax.named_scope("full"):
            return unit(i, br_p, True)

    def noq_body(i, br_p):
        with jax.named_scope("noq"):
            return unit(i, br_p, False)

    def segment(sg, br_p):
        lo = jnp.where(sg == 0, 0, B - L)
        hi = jnp.where(sg == 0, B - L, NU - L)
        br_p = lax.fori_loop(lo, hi, full_body, br_p)

        @pl.when(sg == 0)
        def _():
            wqb_copy.wait()
            xb_copy.wait()
            wob_copy.wait()

        return br_p

    br_p = lax.fori_loop(0, 2, segment, jnp.int32(0))
    lax.fori_loop(NU - L, NU, noq_body, br_p)

    with jax.named_scope("epi"):
        w_last = wo[1, (H - 1) * DH:H * DH, :]
        NS = 2
        RS = SQ // NS
        for r in range(NS):
            rows = pl.ds(r * RS, RS)
            fin = acc[rows, :] + jnp.dot(ol[rows, :], w_last, preferred_element_type=F32)
            obuf[NU - 1, rows, :] = fin.astype(BF16)
            pltpu.make_async_copy(obuf.at[NU - 1, rows, :], out.at[B - 1, rows, pl.ds(D, D)], o_sem).start()
        pltpu.make_async_copy(obuf, obuf, o_sem).wait()


@jax.jit
def pallas_concat_heads__mha_block_cached__mha_block_cached__near_ridge_kernel(
    A_x, A_k_cache, A_v_cache, A_wq, A_wo, B_x, B_k_cache, B_v_cache, B_wq, B_wo):
    any_spec = pl.BlockSpec(memory_space=pl.ANY)
    return pl.pallas_call(
        _kernel,
        in_specs=[any_spec] * 10,
        out_specs=any_spec,
        out_shape=jax.ShapeDtypeStruct((B, SQ, 2 * D), jnp.bfloat16),
        scratch_shapes=[
            pltpu.VMEM((NKV, 2, H, SK, DH), BF16),
            pltpu.VMEM((NU, SQ, D), BF16),
            pltpu.VMEM((2, D, H * DH), BF16),
            pltpu.VMEM((2, H * DH, D), BF16),
            pltpu.VMEM((NQ, H, SQ, DH), BF16),
            pltpu.VMEM((SQ, D), F32),
            pltpu.VMEM((SQ, DH), BF16),
            pltpu.VMEM((NU, SQ, D), BF16),
            pltpu.SemaphoreType.DMA((NKV,)),
            pltpu.SemaphoreType.DMA((8,)),
            pltpu.SemaphoreType.DMA((WC + 1,)),
            pltpu.SemaphoreType.DMA,
            pltpu.SemaphoreType.REGULAR,
        ],
        compiler_params=pltpu.CompilerParams(
            vmem_limit_bytes=120 * 1024 * 1024,
            disable_bounds_checks=True),
    )(A_x, A_k_cache, A_v_cache, A_wq, A_wo, B_x, B_k_cache, B_v_cache, B_wq, B_wo)
```

```python
import jax
import jax.numpy as jnp
from jax import lax
import jax.experimental.pallas as pl
import jax.experimental.pallas.tpu as pltpu

B, SQ, D = 16, 192, 512
H, SK, DH = 32, 512, 128
NU = 2 * B
L = 7
NQ = 8
NKV = 4
HC0 = 4
WC = 2
HC = (H - HC0) // WC
NS = 2
LOG2E = 1.4426950408889634
QSCALE = (DH ** -0.5) * LOG2E
F32 = jnp.float32
BF16 = jnp.bfloat16


def _qproj(x, wq_h):
    q = jnp.dot(x, wq_h, preferred_element_type=F32)
    return (q * QSCALE).astype(BF16)


def _qk(q, k):
    return lax.dot_general(q, k, (((1,), (1,)), ((), ())), preferred_element_type=F32)


def _softmax_pv(s, v):
    m = jnp.max(s, axis=-1, keepdims=True)
    p = jnp.exp2(s - m)
    l = jnp.sum(p, axis=-1, keepdims=True)
    o = jnp.dot(p.astype(BF16), v, preferred_element_type=F32)
    r = pl.reciprocal(l, approx=True)
    r = r * (2.0 - l * r)
    return (o * r).astype(BF16)


def _kernel(xa, ka, va, wqa, woa, xb, kb, vb, wqb, wob, out,
            kvbuf, xbuf, wq, wo, qbuf, acc, ol, obuf, kv_sem, w_sem, wq_sem, o_sem, ord_sem):

    def kv_copies(src_k, src_v, b, s):
        return (pltpu.make_async_copy(src_k.at[b], kvbuf.at[s, 0], kv_sem.at[s]),
                pltpu.make_async_copy(src_v.at[b], kvbuf.at[s, 1], kv_sem.at[s]))

    def start_kv(u):
        s = u & (NKV - 1)
        b = u & (B - 1)

        @pl.when(u < B)
        def _():
            for c in kv_copies(ka, va, b, s):
                c.start()

        @pl.when(jnp.logical_and(u >= B, u < NU))
        def _():
            for c in kv_copies(kb, vb, b, s):
                c.start()

    def wait_kv(s):
        pltpu.make_async_copy(kvbuf.at[s], kvbuf.at[s], kv_sem.at[s]).wait()

    wq0_copy = pltpu.make_async_copy(wqa.at[:, pl.ds(0, HC0 * DH)], wq.at[0, :, pl.ds(0, HC0 * DH)], wq_sem.at[WC])

    def wq_chunk(c):
        cols = pl.ds(pl.multiple_of((HC0 + c * HC) * DH, DH), HC * DH)
        return pltpu.make_async_copy(wqa.at[:, cols], wq.at[0, :, cols], wq_sem.at[c])

    def xa_copy(lo, hi, sem):
        return pltpu.make_async_copy(xa.at[pl.ds(lo, hi - lo)], xbuf.at[pl.ds(lo, hi - lo)], sem)

    x0_copy = xa_copy(0, 1, w_sem.at[0])
    x1_copy = xa_copy(1, 3, w_sem.at[1])
    x2_copy = xa_copy(3, L, w_sem.at[2])
    x3_copy = xa_copy(L, B, w_sem.at[3])
    woa_copy = pltpu.make_async_copy(woa, wo.at[0], w_sem.at[4])
    wqb_copy = pltpu.make_async_copy(wqb, wq.at[1], w_sem.at[5])
    wob_copy = pltpu.make_async_copy(wob, wo.at[1], w_sem.at[6])
    xb_copy = pltpu.make_async_copy(xb, xbuf.at[pl.ds(B, B)], w_sem.at[7])

    def out_copy(u):
        col = pl.multiple_of((u >> 4) * D, D)
        return pltpu.make_async_copy(obuf.at[u], out.at[u & (B - 1), :, pl.ds(col, D)], o_sem)

    def fence():
        pl.semaphore_signal(ord_sem, 1)
        pl.semaphore_wait(ord_sem, 1)

    order = [x0_copy, wq0_copy, x1_copy, x2_copy] + [wq_chunk(c) for c in range(WC)]
    order += list(kv_copies(ka, va, 0, 0)) + [woa_copy, x3_copy]
    for u in range(1, NKV):
        order += list(kv_copies(ka, va, u, u))
    order += [wqb_copy, wob_copy, xb_copy]
    for c in order:
        c.start()
        fence()
    acc[...] = jnp.zeros_like(acc)
    ol[...] = jnp.zeros_like(ol)

    x0_copy.wait()
    wq0_copy.wait()
    for u in range(L):
        if u == 1:
            x1_copy.wait()
        if u == 3:
            x2_copy.wait()
        x = xbuf[u]
        for h in range(HC0):
            qbuf[u, h] = _qproj(x, wq[0, :, h * DH:(h + 1) * DH])

    def qphase(c, carry):
        wq_chunk(c).wait()
        for u in range(L):
            x = xbuf[u]
            for hh in range(HC):
                h = HC0 + c * HC + hh
                col = pl.multiple_of(h * DH, DH)
                qbuf[u, h] = _qproj(x, wq[0, :, pl.ds(col, DH)])
        return carry

    lax.fori_loop(0, WC, qphase, 0)
    woa_copy.wait()
    x3_copy.wait()
    wait_kv(0)

    def unit(i, br_p, with_q):
        kslot = i & (NKV - 1)
        br = i >> 4
        qslot = i & (NQ - 1)

        def o_last():
            fin = acc[...] + jnp.dot(ol[...], wo[br_p, (H - 1) * DH:H * DH, :], preferred_element_type=F32)
            obuf[jnp.maximum(i - 1, 0)] = fin.astype(BF16)

        def o_proj(h, o):
            r = jnp.dot(o, wo[br, h * DH:(h + 1) * DH, :], preferred_element_type=F32)
            if h == 0:
                acc[...] = r
            else:
                acc[...] += r

        def qk(h):
            return _qk(qbuf[qslot, h], kvbuf[kslot, 0, h])

        def pv(h, s):
            return _softmax_pv(s, kvbuf[kslot, 1, h])

        o = {}
        o_last()
        if with_q:
            un = i + L
            br_n = un >> 4
            qslot_n = un & (NQ - 1)
            x = xbuf[un]
            for h in range(H):
                s = qk(h)
                qbuf[qslot_n, h] = _qproj(x, wq[br_n, :, h * DH:(h + 1) * DH])
                o[h] = pv(h, s)
                if h >= 1:
                    o_proj(h - 1, o.pop(h - 1))
        else:
            s = {0: qk(0)}
            for h in range(H):
                if h + 1 < H:
                    s[h + 1] = qk(h + 1)
                o[h] = pv(h, s.pop(h))
                if h >= 1:
                    o_proj(h - 1, o.pop(h - 1))
        ol[...] = o.pop(H - 1)

        start_kv(i + NKV)

        @pl.when(i >= 1)
        def _():
            out_copy(i - 1).start()

        @pl.when(i + 1 < NU)
        def _():
            wait_kv((i + 1) & (NKV - 1))

        return br

    def full_body(i, br_p):
        return unit(i, br_p, True)

    def noq_body(i, br_p):
        return unit(i, br_p, False)

    def segment(sg, br_p):
        lo = jnp.where(sg == 0, 0, B - L)
        hi = jnp.where(sg == 0, B - L, NU - L)
        br_p = lax.fori_loop(lo, hi, full_body, br_p)

        @pl.when(sg == 0)
        def _():
            wqb_copy.wait()
            xb_copy.wait()
            wob_copy.wait()

        return br_p

    br_p = lax.fori_loop(0, 2, segment, jnp.int32(0))
    lax.fori_loop(NU - L, NU, noq_body, br_p)

    w_last = wo[1, (H - 1) * DH:H * DH, :]
    rs = SQ // NS
    for r in range(NS):
        rows = pl.ds(r * rs, rs)
        fin = acc[rows, :] + jnp.dot(ol[rows, :], w_last, preferred_element_type=F32)
        obuf[NU - 1, rows, :] = fin.astype(BF16)
        pltpu.make_async_copy(obuf.at[NU - 1, rows, :], out.at[B - 1, rows, pl.ds(D, D)], o_sem).start()
    pltpu.make_async_copy(obuf, obuf, o_sem).wait()


@jax.jit
def pallas_concat_heads__mha_block_cached__mha_block_cached__near_ridge_kernel(
    A_x, A_k_cache, A_v_cache, A_wq, A_wo, B_x, B_k_cache, B_v_cache, B_wq, B_wo):
    any_spec = pl.BlockSpec(memory_space=pl.ANY)
    return pl.pallas_call(
        _kernel,
        in_specs=[any_spec] * 10,
        out_specs=any_spec,
        out_shape=jax.ShapeDtypeStruct((B, SQ, 2 * D), jnp.bfloat16),
        scratch_shapes=[
            pltpu.VMEM((NKV, 2, H, SK, DH), BF16),
            pltpu.VMEM((NU, SQ, D), BF16),
            pltpu.VMEM((2, D, H * DH), BF16),
            pltpu.VMEM((2, H * DH, D), BF16),
            pltpu.VMEM((NQ, H, SQ, DH), BF16),
            pltpu.VMEM((SQ, D), F32),
            pltpu.VMEM((SQ, DH), BF16),
            pltpu.VMEM((NU, SQ, D), BF16),
            pltpu.SemaphoreType.DMA((NKV,)),
            pltpu.SemaphoreType.DMA((8,)),
            pltpu.SemaphoreType.DMA((WC + 1,)),
            pltpu.SemaphoreType.DMA,
            pltpu.SemaphoreType.REGULAR,
        ],
        compiler_params=pltpu.CompilerParams(
            vmem_limit_bytes=112 * 1024 * 1024,
            disable_bounds_checks=True),
    )(A_x, A_k_cache, A_v_cache, A_wq, A_wo, B_x, B_k_cache, B_v_cache, B_wq, B_wo)
```

```python
import jax
import jax.numpy as jnp
from jax import lax
import jax.experimental.pallas as pl
import jax.experimental.pallas.tpu as pltpu

B, SQ, D = 16, 192, 512
H, SK, DH = 32, 512, 128
NU = 2 * B
L = 7
NQ = 8
NKV = 4
HC0 = 4
WC = 2
HC = (H - HC0) // WC
NS = 4
LOG2E = 1.4426950408889634
QSCALE = (DH ** -0.5) * LOG2E
F32 = jnp.float32
BF16 = jnp.bfloat16


def _qproj(x, wq_h):
    q = jnp.dot(x, wq_h, preferred_element_type=F32)
    return (q * QSCALE).astype(BF16)


def _qk(q, k):
    return lax.dot_general(q, k, (((1,), (1,)), ((), ())), preferred_element_type=F32)


def _softmax_pv(s, v):
    m = jnp.max(s, axis=-1, keepdims=True)
    p = jnp.exp2(s - m)
    l = jnp.sum(p, axis=-1, keepdims=True)
    o = jnp.dot(p.astype(BF16), v, preferred_element_type=F32)
    r = pl.reciprocal(l, approx=True)
    r = r * (2.0 - l * r)
    return (o * r).astype(BF16)


def _kernel(xa, ka, va, wqa, woa, xb, kb, vb, wqb, wob, out,
            kvbuf, xbuf, wq, wo, qbuf, acc, ol, obuf, kv_sem, w_sem, wq_sem, o_sem, ord_sem):

    def kv_copies(src_k, src_v, b, s):
        return (pltpu.make_async_copy(src_k.at[b], kvbuf.at[s, 0], kv_sem.at[s]),
                pltpu.make_async_copy(src_v.at[b], kvbuf.at[s, 1], kv_sem.at[s]))

    def start_kv(u):
        s = u & (NKV - 1)
        b = u & (B - 1)

        @pl.when(u < B)
        def _():
            for c in kv_copies(ka, va, b, s):
                c.start()

        @pl.when(jnp.logical_and(u >= B, u < NU))
        def _():
            for c in kv_copies(kb, vb, b, s):
                c.start()

    def wait_kv(s):
        pltpu.make_async_copy(kvbuf.at[s], kvbuf.at[s], kv_sem.at[s]).wait()

    wq0_copy = pltpu.make_async_copy(wqa.at[:, pl.ds(0, HC0 * DH)], wq.at[0, :, pl.ds(0, HC0 * DH)], wq_sem.at[WC])

    def wq_chunk(c):
        cols = pl.ds(pl.multiple_of((HC0 + c * HC) * DH, DH), HC * DH)
        return pltpu.make_async_copy(wqa.at[:, cols], wq.at[0, :, cols], wq_sem.at[c])

    def xa_copy(lo, hi, sem):
        return pltpu.make_async_copy(xa.at[pl.ds(lo, hi - lo)], xbuf.at[pl.ds(lo, hi - lo)], sem)

    x0_copy = xa_copy(0, 1, w_sem.at[0])
    x1_copy = xa_copy(1, 3, w_sem.at[1])
    x2_copy = xa_copy(3, L, w_sem.at[2])
    x3_copy = xa_copy(L, B, w_sem.at[3])
    woa_copy = pltpu.make_async_copy(woa, wo.at[0], w_sem.at[4])
    wqb_copy = pltpu.make_async_copy(wqb, wq.at[1], w_sem.at[5])
    wob_copy = pltpu.make_async_copy(wob, wo.at[1], w_sem.at[6])
    xb_copy = pltpu.make_async_copy(xb, xbuf.at[pl.ds(B, B)], w_sem.at[7])

    def out_copy(u):
        col = pl.multiple_of((u >> 4) * D, D)
        return pltpu.make_async_copy(obuf.at[u], out.at[u & (B - 1), :, pl.ds(col, D)], o_sem)

    def fence():
        pl.semaphore_signal(ord_sem, 1)
        pl.semaphore_wait(ord_sem, 1)

    order = [x0_copy, wq0_copy, x1_copy, x2_copy] + [wq_chunk(c) for c in range(WC)]
    order += list(kv_copies(ka, va, 0, 0)) + [woa_copy, x3_copy]
    for u in range(1, NKV):
        order += list(kv_copies(ka, va, u, u))
    order += [wqb_copy, wob_copy, xb_copy]
    for c in order:
        c.start()
        fence()
    acc[...] = jnp.zeros_like(acc)
    ol[...] = jnp.zeros_like(ol)

    x0_copy.wait()
    wq0_copy.wait()
    for u in range(L):
        if u == 1:
            x1_copy.wait()
        if u == 3:
            x2_copy.wait()
        x = xbuf[u]
        for h in range(HC0):
            qbuf[u, h] = _qproj(x, wq[0, :, h * DH:(h + 1) * DH])

    def qphase(c, carry):
        wq_chunk(c).wait()
        for u in range(L):
            x = xbuf[u]
            for hh in range(HC):
                h = HC0 + c * HC + hh
                col = pl.multiple_of(h * DH, DH)
                qbuf[u, h] = _qproj(x, wq[0, :, pl.ds(col, DH)])
        return carry

    lax.fori_loop(0, WC, qphase, 0)
    woa_copy.wait()
    x3_copy.wait()
    wait_kv(0)

    def unit(i, br_p, with_q):
        kslot = i & (NKV - 1)
        br = i >> 4
        qslot = i & (NQ - 1)

        def o_last():
            fin = acc[...] + jnp.dot(ol[...], wo[br_p, (H - 1) * DH:H * DH, :], preferred_element_type=F32)
            obuf[jnp.maximum(i - 1, 0)] = fin.astype(BF16)

        def o_proj(h, o):
            r = jnp.dot(o, wo[br, h * DH:(h + 1) * DH, :], preferred_element_type=F32)
            if h == 0:
                acc[...] = r
            else:
                acc[...] += r

        def qk(h):
            return _qk(qbuf[qslot, h], kvbuf[kslot, 0, h])

        def pv(h, s):
            return _softmax_pv(s, kvbuf[kslot, 1, h])

        o = {}

        def o_pair(h):
            og = jnp.concatenate([o.pop(h), o.pop(h + 1)], axis=1)
            r = jnp.dot(og, wo[br, h * DH:(h + 2) * DH, :], preferred_element_type=F32)
            if h == 0:
                acc[...] = r
            else:
                acc[...] += r

        o_last()
        if with_q:
            un = i + L
            br_n = un >> 4
            qslot_n = un & (NQ - 1)
            x = xbuf[un]
            for h in range(H):
                s = qk(h)
                qbuf[qslot_n, h] = _qproj(x, wq[br_n, :, h * DH:(h + 1) * DH])
                o[h] = pv(h, s)
                if h >= 1:
                    o_proj(h - 1, o.pop(h - 1))
        else:
            s = {0: qk(0)}
            for h in range(H):
                if h + 1 < H:
                    s[h + 1] = qk(h + 1)
                o[h] = pv(h, s.pop(h))
                if h == H - 1:
                    o_proj(h - 1, o.pop(h - 1))
                elif h >= 2 and h % 2 == 0:
                    o_pair(h - 2)
        ol[...] = o.pop(H - 1)

        start_kv(i + NKV)

        @pl.when(i >= 1)
        def _():
            out_copy(i - 1).start()

        @pl.when(i + 1 < NU)
        def _():
            wait_kv((i + 1) & (NKV - 1))

        return br

    def full_body(i, br_p):
        return unit(i, br_p, True)

    def noq_body(i, br_p):
        return unit(i, br_p, False)

    def segment(sg, br_p):
        lo = jnp.where(sg == 0, 0, B - L)
        hi = jnp.where(sg == 0, B - L, NU - L)
        br_p = lax.fori_loop(lo, hi, full_body, br_p)

        @pl.when(sg == 0)
        def _():
            wqb_copy.wait()
            xb_copy.wait()
            wob_copy.wait()

        return br_p

    br_p = lax.fori_loop(0, 2, segment, jnp.int32(0))
    lax.fori_loop(NU - L, NU, noq_body, br_p)

    w_last = wo[1, (H - 1) * DH:H * DH, :]
    rs = SQ // NS
    for r in range(NS):
        rows = pl.ds(r * rs, rs)
        fin = acc[rows, :] + jnp.dot(ol[rows, :], w_last, preferred_element_type=F32)
        obuf[NU - 1, rows, :] = fin.astype(BF16)
        pltpu.make_async_copy(obuf.at[NU - 1, rows, :], out.at[B - 1, rows, pl.ds(D, D)], o_sem).start()
    pltpu.make_async_copy(obuf, obuf, o_sem).wait()


@jax.jit
def pallas_concat_heads__mha_block_cached__mha_block_cached__near_ridge_kernel(
    A_x, A_k_cache, A_v_cache, A_wq, A_wo, B_x, B_k_cache, B_v_cache, B_wq, B_wo):
    any_spec = pl.BlockSpec(memory_space=pl.ANY)
    return pl.pallas_call(
        _kernel,
        in_specs=[any_spec] * 10,
        out_specs=any_spec,
        out_shape=jax.ShapeDtypeStruct((B, SQ, 2 * D), jnp.bfloat16),
        scratch_shapes=[
            pltpu.VMEM((NKV, 2, H, SK, DH), BF16),
            pltpu.VMEM((NU, SQ, D), BF16),
            pltpu.VMEM((2, D, H * DH), BF16),
            pltpu.VMEM((2, H * DH, D), BF16),
            pltpu.VMEM((NQ, H, SQ, DH), BF16),
            pltpu.VMEM((SQ, D), F32),
            pltpu.VMEM((SQ, DH), BF16),
            pltpu.VMEM((NU, SQ, D), BF16),
            pltpu.SemaphoreType.DMA((NKV,)),
            pltpu.SemaphoreType.DMA((8,)),
            pltpu.SemaphoreType.DMA((WC + 1,)),
            pltpu.SemaphoreType.DMA,
            pltpu.SemaphoreType.REGULAR,
        ],
        compiler_params=pltpu.CompilerParams(
            vmem_limit_bytes=112 * 1024 * 1024,
            disable_bounds_checks=True),
    )(A_x, A_k_cache, A_v_cache, A_wq, A_wo, B_x, B_k_cache, B_v_cache, B_wq, B_wo)
```
